```python
import os as _os
_os.environ.setdefault("JAX_PLATFORMS", "cpu")
import jax
import jax.numpy as jnp

def _softmax(x, axis=-1):
    return jax.nn.softmax(x, axis=axis)
def _gelu(x):
    return jax.nn.gelu(x, approximate=True)
def _silu(x):
    return jax.nn.silu(x)
def _sigmoid(x):
    return jax.nn.sigmoid(x)
def _layernorm(x, axis=-1, eps=1e-5):
    m = jnp.mean(x, axis=axis, keepdims=True)
    v = jnp.var(x, axis=axis, keepdims=True)
    return (x - m) / jnp.sqrt(v + eps)
def _scatter_add(tgt, idx, src, axis=0):
    return tgt.at[idx].add(src)
def _segment_sum(src, seg, n):
    return jax.ops.segment_sum(src, seg, n)
class _Rng:
    def __init__(self, key):
        self._k = key
    def _next(self):
        self._k, sub = jax.random.split(self._k)
        return sub
    def normal(self, shape):
        return jax.random.normal(self._next(), shape, dtype=jnp.bfloat16)
    def randint(self, lo, hi, shape):
        return jax.random.randint(self._next(), shape, lo, hi, dtype=jnp.int32)
    def uniform(self, shape, lo=0.0, hi=1.0):
        return jax.random.uniform(self._next(), shape, jnp.bfloat16, lo, hi)
    def permutation(self, n):
        return jax.random.permutation(self._next(), n)


kernel_name = 'concat_heads__gqa_block_cached__mha_block_cached__near_ridge'

def setup_inputs():
    _rng = _Rng(jax.random.key(int.from_bytes(__import__("os").urandom(4), "little")))
    _w = (lambda a: (lambda t: t.astype(jnp.bfloat16) if jnp.issubdtype(t.dtype, jnp.floating) else t)(jnp.asarray(a)))
    def _A_setup():
        B, Sq, D = 8, 112, 448
        Hq, Hkv, Sk, Dh = 16, 8, 512, 256
        assert Hq % Hkv == 0, (Hq, Hkv)
        return {
            "x": _w((lambda *s: _rng.normal(s) * 0.8)(B, Sq, D)),
            "k_cache": _w((lambda *s: _rng.normal(s) * 0.8)(B, Hkv, Sk, Dh)),
            "v_cache": _w((lambda *s: _rng.normal(s) * 0.05)(B, Hkv, Sk, Dh)),
            "wq": _w((lambda *s: _rng.normal(s) * 0.8)(D, Hq * Dh) * (D ** -0.5)),
            "wo": _w((lambda *s: _rng.normal(s) * 0.05)(Hq * Dh, D) * ((Hq * Dh) ** -0.5)),
        }
    _A_in = _A_setup()

    def _B_setup():
        B, Sq, D = 8, 112, 448
        H, Sk, Dh = 16, 512, 256
        return {
            "x": _w((lambda *s: _rng.normal(s) * 0.8)(B, Sq, D)),
            "k_cache": _w((lambda *s: _rng.normal(s) * 0.8)(B, H, Sk, Dh)),
            "v_cache": _w((lambda *s: _rng.normal(s) * 0.05)(B, H, Sk, Dh)),
            "wq": _w((lambda *s: _rng.normal(s) * 0.8)(D, H * Dh) * (D ** -0.5)),
            "wo": _w((lambda *s: _rng.normal(s) * 0.05)(H * Dh, D) * ((H * Dh) ** -0.5)),
        }
    _B_in = _B_setup()

    return {
        "A_x": _A_in["x"],
        "A_k_cache": _A_in["k_cache"],
        "A_v_cache": _A_in["v_cache"],
        "A_wq": _A_in["wq"],
        "A_wo": _A_in["wo"],
        "B_x": _B_in["x"],
        "B_k_cache": _B_in["k_cache"],
        "B_v_cache": _B_in["v_cache"],
        "B_wq": _B_in["wq"],
        "B_wo": _B_in["wo"],
    }

def reference(A_x, A_k_cache, A_v_cache, A_wq, A_wo, B_x, B_k_cache, B_v_cache, B_wq, B_wo):
    def _A_ref(x, k_cache, v_cache, wq, wo):
        B, Sq, D = x.shape
        Hq, Dh = 16, 256
        Hkv = k_cache.shape[1]
        rep = Hq // Hkv
        q = (lambda x, *d: x.transpose(*d))((x @ wq).reshape(B, Sq, Hq, Dh), 0, 2, 1, 3)
        k = jnp.repeat(k_cache, rep, axis=1)
        v = jnp.repeat(v_cache, rep, axis=1)
        scores = jnp.einsum("bhqd,bhkd->bhqk", q, k) * (Dh ** -0.5)
        p = _softmax(scores, axis=-1)
        o = jnp.einsum("bhqk,bhkd->bhqd", p, v)
        return (lambda x, *d: x.transpose(*d))(o, 0, 2, 1, 3).reshape(B, Sq, Hq * Dh) @ wo

    def _B_ref(x, k_cache, v_cache, wq, wo):
        B, Sq, D = x.shape
        H, Dh = 16, 256
        q = (lambda x, *d: x.transpose(*d))((x @ wq).reshape(B, Sq, H, Dh), 0, 2, 1, 3)
        scores = jnp.einsum("bhqd,bhkd->bhqk", q, k_cache) * (Dh ** -0.5)
        p = _softmax(scores, axis=-1)
        o = jnp.einsum("bhqk,bhkd->bhqd", p, v_cache)
        return (lambda x, *d: x.transpose(*d))(o, 0, 2, 1, 3).reshape(B, Sq, H * Dh) @ wo

    a = _A_ref(A_x, A_k_cache, A_v_cache, A_wq, A_wo)
    b = _B_ref(B_x, B_k_cache, B_v_cache, B_wq, B_wo)
    return jnp.concatenate([a, b], axis=-1)
```

```python
import jax
import jax.numpy as jnp
from jax import lax
import jax.experimental.pallas as pl
import jax.experimental.pallas.tpu as pltpu

NB, SQ, D, HQ, DH, SK = 8, 112, 448, 16, 256, 512
M = NB * SQ
NG = HQ // 2
NF = 4
NS = 12
NKV = NG + HQ - NF
NMAIN = 2 * NG - NF // 2
FIN0 = (NKV - NS) * 2 * NB
WQ0 = NS * 2 * NB
WO0 = WQ0 + 2 * HQ
NPIECE = M // 128
QH = 6
NQ = (2 * HQ - 2) // QH
NH = 1
HI = 80
QC, M0, MC = (6, 8), (32, 40), (10, 10)
QS = 7
NDOUBLE = 6
EARLY = 2
NT = (((1,), (1,)), ((), ()))
C_EXP2 = (DH ** -0.5) * 1.4426950408889634
BF16, F32 = jnp.bfloat16, jnp.float32


def _ds(i, n, align):
    return pl.ds(i * n if isinstance(i, int) else pl.multiple_of(i * n, align), n)


def _dot(a, b):
    return jnp.dot(a, b, preferred_element_type=F32)


def _dot_nt(a, b):
    return lax.dot_general(a, b, NT, preferred_element_type=F32)


def _softmax_parts(s):
    p = jnp.exp2(s - jnp.max(s, axis=-1, keepdims=True))
    l = jnp.sum(p, axis=-1, keepdims=True)
    r = pl.reciprocal(l, approx=True)
    return p.astype(BF16), r * (2.0 - l * r)


def _kernel(xa, ka, va, wqa, woa, xb, kb, vb, wqb, wob, out,
            x_vm, buf, q_scr, o_scr, o_fin, p_scr, inv_scr, acc, out_vm,
            s_x, s_wq, s_wo, s_kv, s_out):
    def wait_all(view, sem):
        pltpu.make_async_copy(view, view, sem).wait()

    def rows_on(part, n):
        return pl.ds(0, n) if part is None else pl.ds(part * HI, HI if part < NH else n - NH * HI)

    def queue(part):
        return int(part is None or part == NH)

    def cp_x(p, i):
        rows = _ds(i, M // 2, 64)
        return pltpu.make_async_copy((xa, xb)[p].at[rows], x_vm.at[p, rows], s_x.at[2 * p + i])

    def w_at(base, g):
        return buf.at[base + g, pl.ds(0, D)]

    def wait_w(base, g, n, sem):
        wait_all(buf.at[pl.ds(base + g, n), pl.ds(0, D)], sem)

    def start_w(part, src, h, base, g, sem):
        rows = rows_on(part, D)
        pltpu.make_async_copy(src.at[rows, _ds(h, DH, DH)], buf.at[base + g, rows], sem).start(priority=queue(part))

    def start_w_any(part, src_a, src_b, base, g, sem):
        pl.when(g < HQ)(lambda: start_w(part, src_a, g, base, g, sem))
        pl.when((g >= HQ) & (g < 2 * HQ))(lambda: start_w(part, src_b, g - HQ, base, g, sem))

    def start_block(part, src, h, b, blk, sem):
        rows = rows_on(part, SK)
        pltpu.make_async_copy(src.at[b, h, rows], buf.at[blk, rows], sem).start(priority=queue(part))

    def ring(slot, isv, b):
        return (2 * slot + isv) * NB + b

    def fin(b, isv, j):
        return FIN0 + (2 * b + isv) * NF + j

    def start_cell(part, c, isv, only_a=False):
        src_a, src_b = ((ka, kb), (va, vb))[isv]
        if only_a:
            start_block(part, src_a, c >> 3, c & 7, ring(c >> 3, isv, c & 7), s_kv.at[c >> 3])
            return
        f = c - NKV * NB
        u = jnp.where(f >= 0, NKV + (f & 3), c >> 3)
        b = jnp.where(f >= 0, f >> 2, c & 7)
        slot = jnp.where(u >= NS, u - NS, u)
        blk = jnp.where(f >= 0, fin(b, isv, f & 3), ring(slot, isv, b))
        sem = s_kv.at[jnp.where(f >= 0, NS + 2 * b + isv, slot)]
        pl.when(u < NG)(lambda: start_block(part, src_a, u, b, blk, sem))
        pl.when(u >= NG)(lambda: start_block(part, src_b, u - NG, b, blk, sem))

    def spreader(count, start, nblocks):
        calls = iter(range(count))

        def tick():
            n = next(calls)
            for k in range(n * NH * nblocks[0] // count, (n + 1) * NH * nblocks[0] // count):
                start(k % NH, k // NH)
            for k in range(n * nblocks[1] // count, (n + 1) * nblocks[1] // count):
                start(NH, k)
        return tick

    def start_fin(part, b, n):
        isv, j = divmod(n, NF)
        start_block(part, (kb, vb)[isv], HQ - NF + j, b, fin(b, isv, j), s_kv.at[NS + 2 * b + isv])

    def wait_kf(b):
        wait_all(buf.at[pl.ds(fin(b, 0, 0), NF)], s_kv.at[NS + 2 * b])

    def wait_vf(b):
        wait_all(buf.at[pl.ds(fin(b, 1, 0), NF)], s_kv.at[NS + 2 * b + 1])

    def wait_slot(slot):
        wait_all(buf.at[pl.ds(ring(slot, 0, 0), 2 * NB)], s_kv.at[slot])

    def cp_out(t):
        return pltpu.make_async_copy(out_vm.at[_ds(t, 128, 128)], out.at[_ds(t, 128, 128)], s_out.at[t])

    def cp_last(i):
        idx = (pl.ds(M - 128, 128), (pl.ds(0, 384), pl.ds(384, 512))[i])
        return pltpu.make_async_copy(out_vm.at[idx], out.at[idx], s_out.at[NPIECE - 1 + i])

    @pl.loop(0, 2 + 2 * QH)
    def _(g):
        start_w(None, wqa, g, WQ0, g, s_wq.at[jnp.where(g < 2, g, jnp.where(g < 2 + QH, 2, 3))])

        @pl.when(g == 0)
        def _():
            pl.loop(0, 2)(lambda i: cp_x(0, i).start(priority=1))

    for i in range(2):
        cp_x(1, i).start(priority=1)
    acc[...] = jnp.zeros(acc.shape, F32)

    def qproj(g, rows):
        q = _dot(x_vm[g >> 4, rows], w_at(WQ0, g)[...])
        q_scr[g, rows] = (q * C_EXP2).astype(BF16)

    wait_w(WQ0, 0, 1, s_wq.at[0])

    @pl.loop(0, 2)
    def _(i):
        cp_x(0, i).wait()
        qproj(0, _ds(i, M // 2, 64))

    wait_w(WQ0, 1, 1, s_wq.at[1])
    qproj(1, slice(None))

    @pl.loop(0, NQ)
    def _(i):
        @pl.when(i == (HQ - 2) // QH)
        def _():
            cp_x(1, 0).wait()
            cp_x(1, 1).wait()

        wait_w(WQ0, 2 + i * QH, QH, s_wq.at[2 + i])

        def start(part, k):
            if k < QH:
                start_w_any(part, wqa, wqb, WQ0, i * QH + k + 2 + 2 * QH, s_wq.at[jnp.minimum(4 + i, 1 + NQ)])
            elif k < 2 * QH:
                start_w_any(part, woa, wob, WO0, i * QH + k - QH, s_wo.at[(i * QH + k - QH) >> 2])
            else:
                start_cell(part, i * QC[queue(part)] + (k - 2 * QH) // 2, k % 2, only_a=True)

        tick = spreader(QH * QS, start, [2 * QH + 2 * c for c in QC])
        for n in range(QH * QS):
            qproj(i * QH + n // QS + 2, pl.ds(n % QS * (M // QS), M // QS))
            tick()

    for part in range(NH + 1):
        for g in range(NQ * QH, 2 * HQ):
            start_w(part, wob, g - HQ, WO0, g, s_wo.at[g >> 2])
        for hc in range(2 * NQ * QC[queue(part)], 2 * M0[queue(part)]):
            start_cell(part, hc // 2, hc % 2, only_a=True)
    assert M0[0] + NMAIN * MC[0] == NKV * NB + 3 * NF and M0[1] + NMAIN * MC[1] == NKV * NB + 5 * NF

    def slots_of(G):
        is_b = G >= NG
        i0 = jnp.where(is_b, 2 * G - NG, G)
        return [jnp.where(i >= NS, i - NS, i) for i in (i0, jnp.where(is_b, i0 + 1, i0))]

    def wait_pair(G):
        slots = slots_of(G)
        pl.when(G >= NG)(lambda: wait_slot(slots[1]))
        wait_slot(slots[0])

    def piece(G, t):
        w = jnp.concatenate([w_at(WO0, 2 * G + r)[...] for r in range(2)], axis=1)
        acc[t, _ds(G >> 3, D, 64), :] += _dot_nt(w, o_scr[t * 128:(t + 1) * 128, :])

    def pairs(G0, count):
        for u in range(count):
            wait_pair(G0 + u)
        if count % 2 == 0:
            for u in range(0, count, 2):
                wait_w(WO0, 2 * (G0 + u), 4, s_wo.at[(G0 + u) >> 1])
        else:
            pl.when((G0 & 1) == 0)(lambda: wait_w(WO0, 2 * G0, 4, s_wo.at[G0 >> 1]))

        def qk(n):
            u, j = divmod(n, 2 * NB)
            b, r = divmod(j, 2)
            return _dot_nt(q_scr[2 * (G0 + u) + r, b * SQ:(b + 1) * SQ], buf[ring(slots_of(G0 + u)[r], 0, b)])

        def start(part, k):
            start_cell(part, M0[queue(part)] + G0 * MC[queue(part)] + k // 2, k % 2)

        tick = spreader(count * 4 * NB, start, [2 * count * c for c in MC])
        s_next = qk(0)
        for n in range(count * 2 * NB):
            u, j = divmod(n, 2 * NB)
            b, r = divmod(j, 2)
            G = G0 + u
            s = s_next
            if n + 1 < count * 2 * NB:
                s_next = qk(n + 1)
            tick()
            p, inv = _softmax_parts(s)
            if r == 1 and b >= 3:
                piece(G, b - 3)
            if r == 1 and b < 2 and u > 0:
                piece(G - 1, NPIECE - 2 + b)
            o = _dot(p, buf[ring(slots_of(G)[r], 1, b)]) * inv
            o_scr[b * SQ:(b + 1) * SQ, r * DH:(r + 1) * DH] = o.astype(BF16)
            tick()
        piece(G0 + count - 1, NPIECE - 2)
        piece(G0 + count - 1, NPIECE - 1)

    if NDOUBLE:
        pl.loop(0, NDOUBLE)(lambda i: pairs(2 * i, 2))
    pl.loop(2 * NDOUBLE, NMAIN)(lambda G: pairs(G, 1))

    def qk_fin(b, j):
        return _dot_nt(q_scr[2 * NMAIN + j, _ds(b, SQ, 16)], buf[fin(b, 0, j)])

    def put_p(j, s):
        p, inv = _softmax_parts(s)
        p_scr[j] = p
        inv_scr[j] = jnp.broadcast_to(inv, (SQ, 128))

    def pv_fin(b, j, p=None, inv=None):
        if p is None:
            p, inv = p_scr[j], jnp.concatenate([inv_scr[j]] * (DH // 128), axis=1)
        o_fin[_ds(b, SQ, 16), j * DH:(j + 1) * DH] = (_dot(p, buf[fin(b, 1, j)]) * inv).astype(BF16)

    def emit(t, c0=0, c1=2 * D):
        out_vm[_ds(t, 128, 128), c0:c1] = acc[t, c0:c1, :].T.astype(BF16)

    def oproj_fin(t, j):
        return _dot_nt(w_at(WO0, 2 * NMAIN + j)[...], o_fin[_ds(t, 128, 128), j * DH:(j + 1) * DH])

    def qk_stage(b, s, tick=lambda: None):
        t = b - 2
        r = acc[t, D:, :]
        for j in range(NF):
            s_cur = s
            if j + 1 < NF:
                s = qk_fin(b, j + 1)
            tick()
            put_p(j, s_cur)
            r += oproj_fin(t, j)
        acc[t, D:, :] = r

    wait_w(WO0, 2 * NMAIN, NF, s_wo.at[NMAIN // 2])
    wait_kf(0)
    wait_vf(0)
    wait_kf(1)
    tick = spreader(3 * NF, lambda part, n: start_fin(part, 3 + 2 * queue(part), n), [2 * NF] * 2)
    s_next = qk_fin(1, 0)
    for n in range(2 * NF):
        s = s_next
        if n + 1 < 2 * NF:
            s_next = qk_fin(1 - (n + 1) // NF, (n + 1) % NF)
        tick()
        if n < NF - 1:
            put_p(n, s)
        elif n == NF - 1:
            s_last = s
        else:
            p, inv = _softmax_parts(s)
            if n == NF:
                put_p(NF - 1, s_last)
            if n > NF:
                pv_fin(0, n - NF - 1, *prev)
            tick()
            prev = (p, inv)
    pv_fin(0, NF - 1, *prev)
    emit(NPIECE - 1, 0, 384)

    @pl.loop(1, NB - 2)
    def _(b):
        wait_vf(b)
        wait_kf(b + 1)
        emit(jnp.maximum(b - 2, 0))

        def start(part, n):
            nb = b + 3 + 2 * queue(part)
            pl.when(nb < NB)(lambda: start_fin(part, nb, n))

        tick = spreader(2 * NF, start, [2 * NF] * 2)
        s = qk_fin(b + 1, 0)
        for j in range(NF):
            tick()
            pv_fin(b, j)
        qk_stage(b + 1, s, tick)

    wait_vf(NB - 2)
    emit(NPIECE - 3)
    for j in range(NF):
        pv_fin(NB - 2, j)
    wait_kf(NB - 1)
    for t in range(EARLY):
        cp_out(t).start()
    qk_stage(NB - 1, qk_fin(NB - 1, 0))

    wait_vf(NB - 1)
    cp_last(0).start()
    for t in range(EARLY, NPIECE - 2):
        cp_out(t).start()
    emit(NPIECE - 2)
    cp_out(NPIECE - 2).start()
    for j in range(NF):
        pv_fin(NB - 1, j)
    r = acc[NPIECE - 1, D:, :]
    for j in range(NF):
        r += oproj_fin(NPIECE - 1, j)
    r = jnp.concatenate([acc[NPIECE - 1, 384:D, :], r], axis=0)
    out_vm[M - 128:, 384:] = r.T.astype(BF16)
    cp_last(1).start()

    for t in range(NPIECE - 1):
        cp_out(t).wait()
    cp_last(0).wait()
    cp_last(1).wait()


@jax.jit
def pallas_concat_heads__gqa_block_cached__mha_block_cached__near_ridge_kernel(
        A_x, A_k_cache, A_v_cache, A_wq, A_wo, B_x, B_k_cache, B_v_cache, B_wq, B_wo):
    out = pl.pallas_call(
        _kernel,
        out_shape=jax.ShapeDtypeStruct((M, 2 * D), BF16),
        in_specs=[pl.BlockSpec(memory_space=pl.ANY)] * 10,
        out_specs=pl.BlockSpec(memory_space=pl.ANY),
        scratch_shapes=[
            pltpu.VMEM((2, M, D), BF16),
            pltpu.VMEM((WO0 + 2 * HQ, SK, DH), BF16),
            pltpu.VMEM((2 * HQ, M, DH), BF16),
            pltpu.VMEM((M, 2 * DH), BF16),
            pltpu.VMEM((M, NF * DH), BF16),
            pltpu.VMEM((NF, SQ, SK), BF16),
            pltpu.VMEM((NF, SQ, 128), F32),
            pltpu.VMEM((NPIECE, 2 * D, 128), F32),
            pltpu.VMEM((M, 2 * D), BF16),
            pltpu.SemaphoreType.DMA((4,)),
            pltpu.SemaphoreType.DMA((2 + NQ,)),
            pltpu.SemaphoreType.DMA((NG,)),
            pltpu.SemaphoreType.DMA((NS + 2 * NB,)),
            pltpu.SemaphoreType.DMA((NPIECE + 1,)),
        ],
        compiler_params=pltpu.CompilerParams(
            vmem_limit_bytes=120 * 2**20, disable_bounds_checks=True, disable_semaphore_checks=True),
    )(A_x.reshape(M, D), A_k_cache, A_v_cache, A_wq, A_wo.T,
      B_x.reshape(M, D), B_k_cache, B_v_cache, B_wq, B_wo.T)
    return out.reshape(NB, SQ, 2 * D)
```

```python
import jax
import jax.numpy as jnp
from jax import lax
import jax.experimental.pallas as pl
import jax.experimental.pallas.tpu as pltpu

NB, SQ, D, HQ, DH, SK = 8, 112, 448, 16, 256, 512
M = NB * SQ
NPIECE = M // 128
NG = HQ // 2
NF = 4
NKV = NG + HQ - NF
NMAIN = 2 * NG - NF // 2
NDOUBLE = 6
NS = 12

FIN0 = (NKV - NS) * 2 * NB
WQ0 = NS * 2 * NB
WO0 = WQ0 + 2 * HQ
OUT0 = NF * DH

XCUT = (0, 256, 576, M)
Q0, QH, NQ = 3, 5, 5
QS = 7
OH = 7

NH, HI = 2, 96
QC, C2, C1 = (6, 4), (20, 24), (11, 8)
LEAD = 4
STAGES = (
    (0, 6, 0, 10, 24), (6, 9, 0, 12, 12), (9, 12, 0, 14, 10),
    (12, 14, 0, 16, 8), (14, 15, 3, 16, 4), (15, 16, 6, 16, 1))

C_EXP2 = (DH ** -0.5) * 1.4426950408889634
BF16, F32 = jnp.bfloat16, jnp.float32


def _ds(i, n, align):
    return pl.ds(i * n if isinstance(i, int) else pl.multiple_of(i * n, align), n)


def _dot(a, b):
    return jnp.dot(a, b, preferred_element_type=F32)


def _dot_nt(a, b):
    return lax.dot_general(a, b, (((1,), (1,)), ((), ())), preferred_element_type=F32)


def _softmax_parts(s):
    p = jnp.exp2(s - jnp.max(s, axis=-1, keepdims=True))
    l = jnp.sum(p, axis=-1, keepdims=True)
    r = pl.reciprocal(l, approx=True)
    return p.astype(BF16), r * (2.0 - l * r)


def _queue(part):
    return int(part is None or part == NH)


def _rows(part, n):
    return pl.ds(0, n) if part is None else pl.ds(part * HI, HI if part < NH else n - NH * HI)


def _spreader(count, start, nblocks):
    calls = iter(range(count))

    def tick():
        n = next(calls, None)
        if n is None:
            return
        for k in range(n * NH * nblocks[0] // count, (n + 1) * NH * nblocks[0] // count):
            start(k % NH, k // NH)
        for k in range(n * nblocks[1] // count, (n + 1) * nblocks[1] // count):
            start(NH, k)
    return tick


def _ring(slot, isv, b):
    return (2 * slot + isv) * NB + b


def _fin(b, isv, j):
    return FIN0 + (2 * b + isv) * NF + j


def _wait_all(view, sem):
    pltpu.make_async_copy(view, view, sem).wait()


def _kernel(xa, ka, va, wqa, woa, xb, kb, vb, wqb, wob, out,
            x_vm, buf, q_vm, q_fin, o_vm, fin_vm, p_vm, inv_vm, acc,
            s_x, s_wq, s_wo, s_kv, s_out):
    nx = len(XCUT) - 1

    def cp_x(i):
        if i == nx:
            return pltpu.make_async_copy(xb, x_vm.at[1], s_x.at[i])
        rows = pl.ds(XCUT[i], XCUT[i + 1] - XCUT[i])
        return pltpu.make_async_copy(xa.at[rows], x_vm.at[0, rows], s_x.at[i])

    def weight(base, g):
        return buf[base + g, pl.ds(0, D)]

    def weights(base, g, n):
        return jnp.concatenate([weight(base, g + r) for r in range(n)], axis=1)

    def wait_w(base, g, n, sem):
        _wait_all(buf.at[pl.ds(base + g, n), pl.ds(0, D)], sem)

    def start_w(part, src_a, src_b, base, g, sem):
        def go(src, h):
            rows = _rows(part, D)
            pltpu.make_async_copy(src.at[rows, _ds(h, DH, DH)], buf.at[base + g, rows],
                                  sem).start(priority=_queue(part))
        pl.when(g < HQ)(lambda: go(src_a, g))
        pl.when((g >= HQ) & (g < 2 * HQ))(lambda: go(src_b, g - HQ))

    def start_kv(part, src, b, h, blk, sem):
        rows = _rows(part, SK)
        pltpu.make_async_copy(src.at[b, h, rows], buf.at[blk, rows], sem).start(priority=_queue(part))

    def start_fin(part, b, isv, j):
        h, blk = HQ - NF + j, _fin(b, isv, j)
        if part == NH:
            h, blk = pl.ds(h, NF), pl.ds(blk, NF)
        start_kv(part, (kb, vb)[isv], b, h, blk, s_kv.at[NS + 2 * b + isv])

    def start_nth(part, first, k, only_a=False):
        if part < NH:
            c, isv = first + k // 2, k % 2
        elif k % 4 == 0:
            c, isv = first + k // 8 * 4, k // 4 % 2
        else:
            return
        u, b = c >> 3, c & 7
        slot = jnp.where(u >= NS, u - NS, u)

        def go(src, h):
            bs, blk = b, _ring(slot, isv, b)
            if part == NH:
                bs, blk = pl.ds(bs, 4), pl.ds(blk, 4)
            start_kv(part, src, bs, h, blk, s_kv.at[slot])

        if only_a:
            return go((ka, va)[isv], u)
        pl.when(u < NG)(lambda: go((ka, va)[isv], u))
        pl.when((u >= NG) & (u < NKV))(lambda: go((kb, vb)[isv], u - NG))
        pl.when(u >= NKV)(lambda: start_fin(part, (c - NKV * NB) >> 2, isv, 0 if part == NH else c & 3))

    def cp_out(t):
        rows = pl.ds(t * 128, 128)
        return pltpu.make_async_copy(fin_vm.at[rows, pl.ds(OUT0, 2 * D)], out.at[rows], s_out.at[t])

    def cp_last(i):
        rows, (c0, n) = pl.ds(M - 128, 128), ((0, 384), (384, 512))[i]
        return pltpu.make_async_copy(fin_vm.at[rows, pl.ds(OUT0 + c0, n)], out.at[rows, pl.ds(c0, n)],
                                     s_out.at[NPIECE - 1 + i])

    pltpu.make_async_copy(wqa.at[:, pl.ds(0, DH)], buf.at[WQ0, pl.ds(0, D)], s_wq.at[0]).start()

    @pl.loop(0, nx - 1 + Q0 + 2 * QH)
    def _(n):
        g = n - nx + 1
        sem = s_wq.at[jnp.where(g < Q0, 1, jnp.where(g < Q0 + QH, 2, 3))]
        pl.when(g > 0)(lambda: start_w(None, wqa, wqb, WQ0, g, sem))
        for i in range(nx + 1):
            pl.when(n == (i if i < nx else nx - 1 + Q0 + QH))(lambda: cp_x(i).start(priority=1))

    acc[...] = jnp.zeros(acc.shape, F32)

    def qproj(g, rows):
        return (_dot(x_vm[g >> 4, rows], weight(WQ0, g)) * C_EXP2).astype(BF16)

    wait_w(WQ0, 0, 1, s_wq.at[0])
    for i in range(nx):
        cp_x(i).wait()
        q_vm[0, XCUT[i]:XCUT[i + 1]] = qproj(0, slice(XCUT[i], XCUT[i + 1]))
    wait_w(WQ0, 1, Q0 - 1, s_wq.at[1])
    for g in range(1, Q0):
        q_vm[g] = qproj(g, slice(None))

    @pl.loop(0, NQ)
    def _(i):
        pl.when(i == (HQ - Q0) // QH)(lambda: cp_x(nx).wait())
        wait_w(WQ0, Q0 + i * QH, QH, s_wq.at[2 + i])

        def start(part, k):
            if k < 2 * QH:
                start_w(part, wqa, wqb, WQ0, Q0 + (2 * i + 2) * QH + k,
                        s_wq.at[jnp.minimum(4 + 2 * i + k // QH, 2 + NQ)])
            elif k < 2 * QH + OH:
                g = i * OH + k - 2 * QH
                start_w(part, woa, wob, WO0, g, s_wo.at[jnp.minimum(g >> 2, NG - 1)])
            else:
                start_nth(part, i * QC[_queue(part)], k - 2 * QH - OH, only_a=True)

        tick = _spreader(QH * QS, start, [2 * QH + OH + 2 * c for c in QC])
        for n in range(QH * QS):
            g, rows = Q0 + i * QH + n // QS, pl.ds(n % QS * (M // QS), M // QS)
            q_vm[g, rows] = qproj(g, rows)
            tick()

    assert Q0 + NQ * QH == 2 * NMAIN and NQ * OH >= 2 * HQ
    wait_w(WQ0, 2 * NMAIN, NF, s_wq.at[2 + NQ])

    def slots_of(G):
        is_b = G >= NG
        u = jnp.where(is_b, 2 * G - NG, G)
        return [jnp.where(i >= NS, i - NS, i) for i in (u, jnp.where(is_b, u + 1, u))]

    def wait_slot(slot):
        _wait_all(buf.at[pl.ds(_ring(slot, 0, 0), 2 * NB)], s_kv.at[slot])

    def piece(G, t):
        acc[t, _ds(G >> 3, D, 64), :] += _dot_nt(weights(WO0, 2 * G, 2), o_vm[t * 128:(t + 1) * 128, :])

    def pairs(G0, count, step, first, cells):
        for u in range(count):
            slots = slots_of(G0 + u)
            pl.when(G0 + u >= NG)(lambda: wait_slot(slots[1]))
            wait_slot(slots[0])
        if count == 2:
            wait_w(WO0, 2 * G0, 4, s_wo.at[G0 >> 1])
        else:
            pl.when((G0 & 1) == 0)(lambda: wait_w(WO0, 2 * G0, 4, s_wo.at[G0 >> 1]))

        def qk(n):
            u, j = divmod(n, 2 * NB)
            b, r = divmod(j, 2)
            return _dot_nt(q_vm[2 * (G0 + u) + r, b * SQ:(b + 1) * SQ], buf[_ring(slots_of(G0 + u)[r], 0, b)])

        tick = _spreader(count * 4 * NB, lambda part, k: start_nth(part, first[_queue(part)], k),
                         [2 * c for c in cells])
        for j in range(NF):
            q_fin[j, _ds(step, SQ, 16)] = qproj(2 * NMAIN + j, _ds(step, SQ, 16))
        s_next = qk(0)
        for n in range(count * 2 * NB):
            u, j = divmod(n, 2 * NB)
            b, r = divmod(j, 2)
            s = s_next
            if n + 1 < count * 2 * NB:
                s_next = qk(n + 1)
            tick()
            p, inv = _softmax_parts(s)
            if r == 1 and b >= 3:
                piece(G0 + u, b - 3)
            if r == 1 and b < 2 and u > 0:
                piece(G0 + u - 1, NPIECE - 2 + b)
            o = _dot(p, buf[_ring(slots_of(G0 + u)[r], 1, b)]) * inv
            o_vm[b * SQ:(b + 1) * SQ, r * DH:(r + 1) * DH] = o.astype(BF16)
            tick()
        piece(G0 + count - 1, NPIECE - 2)
        piece(G0 + count - 1, NPIECE - 1)

    nsingle = NMAIN - 2 * NDOUBLE
    m0 = [NQ * c for c in QC]
    m1 = [m + NDOUBLE * c for m, c in zip(m0, C2)]
    m2 = [m + nsingle * c - NKV * NB for m, c in zip(m1, C1)]
    assert NDOUBLE + nsingle == NB and all(m % NF == 0 for m in m2)
    for q in range(2):
        assert all(m0[q] + i * C2[q] >= NB * max(2 * i + 2, 4 * i + 4 - NG) for i in range(NDOUBLE))
        assert all(m1[q] + i * C1[q] >= NB * (4 * NDOUBLE - NG + 2 * i + 2) for i in range(nsingle))
    pl.loop(0, NDOUBLE)(lambda i: pairs(2 * i, 2, i, [m + i * c for m, c in zip(m0, C2)], C2))
    pl.loop(0, nsingle)(
        lambda i: pairs(2 * NDOUBLE + i, 1, NDOUBLE + i, [m + i * c for m, c in zip(m1, C1)], C1))

    def qk_fin(b, j):
        return _dot_nt(q_fin[j, b * SQ:(b + 1) * SQ], buf[_fin(b, 0, j)])

    def pv_fin(b, j, p, inv):
        fin_vm[b * SQ:(b + 1) * SQ, j * DH:(j + 1) * DH] = (_dot(p, buf[_fin(b, 1, j)]) * inv).astype(BF16)

    def oproj_fin(t):
        return acc[t, D:, :] + _dot_nt(weights(WO0, 2 * NMAIN, NF), fin_vm[t * 128:(t + 1) * 128, :OUT0])

    def emit(t, n=2 * D):
        fin_vm[t * 128:(t + 1) * 128, OUT0:OUT0 + n] = acc[t, :n, :].T.astype(BF16)

    issued = [2 * m2[_queue(part)] for part in range(NH + 1)]

    def start_late(part, _):
        b, isv, j = issued[part] // (2 * NF), issued[part] // NF % 2, issued[part] % NF
        if part < NH or j == 0:
            start_fin(part, b, isv, j)
        issued[part] += 1

    wait_w(WO0, 2 * NMAIN, NF, s_wo.at[NMAIN // 2])
    done = emitted = sent = 0
    for lo, hi, send, nxt, ticks in STAGES:
        assert min(issued) >= hi * NF
        for n in range(lo, hi):
            _wait_all(buf.at[pl.ds(_fin(n // 2, n % 2, 0), NF)], s_kv.at[NS + n])
        if hi == 2 * NB:
            cp_last(0).start()

        def flush():
            nonlocal sent
            while sent < min(send, emitted):
                cp_out(sent).start()
                sent += 1

        def finish():
            nonlocal emitted
            while emitted < done:
                emit(emitted)
                emitted += 1
            flush()
            if lo == 0:
                emit(NPIECE - 1, 384)

        flush()
        tick = _spreader(ticks, start_late,
                         [nxt * NF - issued[0], min(nxt + LEAD, 2 * NB) * NF - issued[NH]])
        if lo % 2:
            for j in range(NF):
                tick()
                pv_fin(lo // 2, j, p_vm[j], jnp.concatenate([inv_vm[j]] * (DH // 128), axis=1))
                if j == 1:
                    finish()
        units = [(n // 2, j) for n in range(lo, hi) if n % 2 == 0 for j in range(NF)]
        have = (lo + 1) // 2
        limit = (hi - 1) // 2 - 1
        if units:
            s_next = qk_fin(*units[0])
        for i, (b, j) in enumerate(units):
            s = s_next
            if i + 1 < len(units):
                s_next = qk_fin(*units[i + 1])
            tick()
            p, inv = _softmax_parts(s)
            keep = 2 * b + 1 == hi
            if keep:
                p_vm[j] = p
                inv_vm[j] = jnp.broadcast_to(inv, (SQ, 128))
            if j == NF - 1 and done < min(have - 1, limit):
                acc[done, D:, :] = oproj_fin(done)
                done += 1
            if not keep:
                pv_fin(b, j, p, inv)
                have += j == NF - 1
            if i == 1 and lo % 2 == 0:
                finish()
            tick()
        while done < limit:
            acc[done, D:, :] = oproj_fin(done)
            done += 1
    assert done == emitted == sent == NPIECE - 1
    r = jnp.concatenate([acc[NPIECE - 1, 384:D, :], oproj_fin(NPIECE - 1)], axis=0)
    fin_vm[M - 128:, OUT0 + 384:] = r.T.astype(BF16)
    cp_last(1).start()

    for t in range(NPIECE - 1):
        cp_out(t).wait()
    cp_last(0).wait()
    cp_last(1).wait()


@jax.jit
def pallas_concat_heads__gqa_block_cached__mha_block_cached__near_ridge_kernel(
    A_x: jax.Array,
    A_k_cache: jax.Array,
    A_v_cache: jax.Array,
    A_wq: jax.Array,
    A_wo: jax.Array,
    B_x: jax.Array,
    B_k_cache: jax.Array,
    B_v_cache: jax.Array,
    B_wq: jax.Array,
    B_wo: jax.Array,
):
    out = pl.pallas_call(
        _kernel,
        out_shape=jax.ShapeDtypeStruct((M, 2 * D), BF16),
        in_specs=[pl.BlockSpec(memory_space=pl.ANY)] * 10,
        out_specs=pl.BlockSpec(memory_space=pl.ANY),
        scratch_shapes=[
            pltpu.VMEM((2, M, D), BF16),
            pltpu.VMEM((WO0 + 2 * HQ, SK, DH), BF16),
            pltpu.VMEM((2 * NMAIN, M, DH), BF16),
            pltpu.VMEM((NF, M, DH), BF16),
            pltpu.VMEM((M, 2 * DH), BF16),
            pltpu.VMEM((M, OUT0 + 2 * D), BF16),
            pltpu.VMEM((NF, SQ, SK), BF16),
            pltpu.VMEM((NF, SQ, 128), F32),
            pltpu.VMEM((NPIECE, 2 * D, 128), F32),
            pltpu.SemaphoreType.DMA((len(XCUT),)),
            pltpu.SemaphoreType.DMA((3 + NQ,)),
            pltpu.SemaphoreType.DMA((NG,)),
            pltpu.SemaphoreType.DMA((NS + 2 * NB,)),
            pltpu.SemaphoreType.DMA((NPIECE + 1,)),
        ],
        compiler_params=pltpu.CompilerParams(
            vmem_limit_bytes=120 * 2**20, disable_bounds_checks=True, disable_semaphore_checks=True),
    )(A_x.reshape(M, D), A_k_cache, A_v_cache, A_wq, A_wo.T,
      B_x.reshape(M, D), B_k_cache, B_v_cache, B_wq, B_wo.T)
    return out.reshape(NB, SQ, 2 * D)
```

```python
import jax
import jax.numpy as jnp
from jax import lax
import jax.experimental.pallas as pl
import jax.experimental.pallas.tpu as pltpu

NB, SQ, D, HQ, DH, SK = 8, 112, 448, 16, 256, 512
M = NB * SQ
NPIECE = M // 128
NG = HQ // 2
NF = 4
NKV = NG + HQ - NF
NMAIN = 2 * NG - NF // 2
NDOUBLE = 6
NS = 12

FIN0 = (NKV - NS) * 2 * NB
WQ0 = NS * 2 * NB
WO0 = WQ0 + 2 * HQ
OUT0 = NF * DH

XCUT = (0, 256, 576, M)
Q0, QH, NQ = 3, 5, 5
QS = 7
OH = 7

NH, HI = 2, 96
QC, C2, C1 = (6, 4), (20, 24), (11, 8)
LEAD = 4
STAGES = (
    (0, 6, 0, 10, 24), (6, 9, 0, 12, 12), (9, 12, 0, 14, 10),
    (12, 14, 0, 16, 8), (14, 15, 3, 16, 4), (15, 16, 6, 16, 1))

C_EXP2 = (DH ** -0.5) * 1.4426950408889634
BF16, F32 = jnp.bfloat16, jnp.float32


def _ds(i, n, align):
    return pl.ds(i * n if isinstance(i, int) else pl.multiple_of(i * n, align), n)


def _dot(a, b):
    return jnp.dot(a, b, preferred_element_type=F32)


def _dot_nt(a, b):
    return lax.dot_general(a, b, (((1,), (1,)), ((), ())), preferred_element_type=F32)


def _softmax_parts(s):
    p = jnp.exp2((s - jnp.max(s, axis=-1, keepdims=True)) * C_EXP2)
    l = jnp.sum(p, axis=-1, keepdims=True)
    r = pl.reciprocal(l, approx=True)
    return p.astype(BF16), r * (2.0 - l * r)


def _queue(part):
    return int(part is None or part == NH)


def _rows(part, n):
    return pl.ds(0, n) if part is None else pl.ds(part * HI, HI if part < NH else n - NH * HI)


def _spreader(count, start, nblocks):
    calls = iter(range(count))

    def tick():
        n = next(calls, None)
        if n is None:
            return
        for k in range(n * NH * nblocks[0] // count, (n + 1) * NH * nblocks[0] // count):
            start(k % NH, k // NH)
        for k in range(n * nblocks[1] // count, (n + 1) * nblocks[1] // count):
            start(NH, k)
    return tick


def _ring(slot, isv, b):
    return (2 * slot + isv) * NB + b


def _fin(b, isv, j):
    return FIN0 + (2 * b + isv) * NF + j


def _wait_all(view, sem):
    pltpu.make_async_copy(view, view, sem).wait()


def _kernel(xa, ka, va, wqa, woa, xb, kb, vb, wqb, wob, out,
            x_vm, buf, q_vm, q_fin, o_vm, fin_vm, p_vm, inv_vm, acc,
            s_x, s_wq, s_wo, s_kv, s_out):
    nx = len(XCUT) - 1

    def cp_x(i):
        if i == nx:
            return pltpu.make_async_copy(xb, x_vm.at[1], s_x.at[i])
        rows = pl.ds(XCUT[i], XCUT[i + 1] - XCUT[i])
        return pltpu.make_async_copy(xa.at[rows], x_vm.at[0, rows], s_x.at[i])

    def weight(base, g):
        return buf[base + g, pl.ds(0, D)]

    def wait_w(base, g, n, sem):
        _wait_all(buf.at[pl.ds(base + g, n), pl.ds(0, D)], sem)

    def start_w(part, src_a, src_b, base, g, sem):
        def go(src, h):
            rows = _rows(part, D)
            pltpu.make_async_copy(src.at[rows, _ds(h, DH, DH)], buf.at[base + g, rows],
                                  sem).start(priority=_queue(part))
        pl.when(g < HQ)(lambda: go(src_a, g))
        pl.when((g >= HQ) & (g < 2 * HQ))(lambda: go(src_b, g - HQ))

    def start_kv(part, src, b, h, blk, sem):
        rows = _rows(part, SK)
        pltpu.make_async_copy(src.at[b, h, rows], buf.at[blk, rows], sem).start(priority=_queue(part))

    def start_fin(part, b, isv, j):
        h, blk = HQ - NF + j, _fin(b, isv, j)
        if part == NH:
            h, blk = pl.ds(h, NF), pl.ds(blk, NF)
        start_kv(part, (kb, vb)[isv], b, h, blk, s_kv.at[NS + 2 * b + isv])

    def start_nth(part, first, k, only_a=False):
        if part < NH:
            c, isv = first + k // 2, k % 2
        elif k % 4 == 0:
            c, isv = first + k // 8 * 4, k // 4 % 2
        else:
            return
        u, b = c >> 3, c & 7
        slot = jnp.where(u >= NS, u - NS, u)

        def go(src, h):
            bs, blk = b, _ring(slot, isv, b)
            if part == NH:
                bs, blk = pl.ds(bs, 4), pl.ds(blk, 4)
            start_kv(part, src, bs, h, blk, s_kv.at[slot])

        if only_a:
            return go((ka, va)[isv], u)
        pl.when(u < NG)(lambda: go((ka, va)[isv], u))
        pl.when((u >= NG) & (u < NKV))(lambda: go((kb, vb)[isv], u - NG))
        pl.when(u >= NKV)(lambda: start_fin(part, (c - NKV * NB) >> 2, isv, 0 if part == NH else c & 3))

    def cp_out(t):
        rows = pl.ds(t * 128, 128)
        return pltpu.make_async_copy(fin_vm.at[rows, pl.ds(OUT0, 2 * D)], out.at[rows], s_out.at[t])

    def cp_last(i):
        rows, (c0, n) = pl.ds(M - 128, 128), ((0, 384), (384, 256), (640, 256))[i]
        return pltpu.make_async_copy(fin_vm.at[rows, pl.ds(OUT0 + c0, n)], out.at[rows, pl.ds(c0, n)],
                                     s_out.at[NPIECE - 1 + i])

    pltpu.make_async_copy(wqa.at[:, pl.ds(0, DH)], buf.at[WQ0, pl.ds(0, D)], s_wq.at[0]).start()

    @pl.loop(0, nx - 1 + Q0 + 2 * QH)
    def _(n):
        g = n - nx + 1
        sem = s_wq.at[jnp.where(g < Q0, 1, jnp.where(g < Q0 + QH, 2, 3))]
        pl.when(g > 0)(lambda: start_w(None, wqa, wqb, WQ0, g, sem))
        for i in range(nx + 1):
            pl.when(n == (i if i < nx else nx - 1 + Q0 + QH))(lambda: cp_x(i).start(priority=1))

    acc[...] = jnp.zeros(acc.shape, F32)

    def qproj(g, rows):
        return _dot(x_vm[g >> 4, rows], weight(WQ0, g)).astype(BF16)

    wait_w(WQ0, 0, 1, s_wq.at[0])
    for i in range(nx):
        cp_x(i).wait()
        q_vm[0, XCUT[i]:XCUT[i + 1]] = qproj(0, slice(XCUT[i], XCUT[i + 1]))
    wait_w(WQ0, 1, Q0 - 1, s_wq.at[1])
    for g in range(1, Q0):
        q_vm[g] = qproj(g, slice(None))

    @pl.loop(0, NQ)
    def _(i):
        pl.when(i == (HQ - Q0) // QH)(lambda: cp_x(nx).wait())
        wait_w(WQ0, Q0 + i * QH, QH, s_wq.at[2 + i])

        def start(part, k):
            if k < 2 * QH:
                start_w(part, wqa, wqb, WQ0, Q0 + (2 * i + 2) * QH + k,
                        s_wq.at[jnp.minimum(4 + 2 * i + k // QH, 2 + NQ)])
            elif k < 2 * QH + OH:
                g = i * OH + k - 2 * QH
                start_w(part, woa, wob, WO0, g, s_wo.at[jnp.minimum(g >> 2, NG - 1)])
            else:
                start_nth(part, i * QC[_queue(part)], k - 2 * QH - OH, only_a=True)

        tick = _spreader(QH * QS, start, [2 * QH + OH + 2 * c for c in QC])
        for n in range(QH * QS):
            g, rows = Q0 + i * QH + n // QS, pl.ds(n % QS * (M // QS), M // QS)
            q_vm[g, rows] = qproj(g, rows)
            tick()

    assert Q0 + NQ * QH == 2 * NMAIN and NQ * OH >= 2 * HQ
    wait_w(WQ0, 2 * NMAIN, NF, s_wq.at[2 + NQ])

    def slots_of(G):
        is_b = G >= NG
        u = jnp.where(is_b, 2 * G - NG, G)
        return [jnp.where(i >= NS, i - NS, i) for i in (u, jnp.where(is_b, u + 1, u))]

    def wait_slot(slot):
        _wait_all(buf.at[pl.ds(_ring(slot, 0, 0), 2 * NB)], s_kv.at[slot])

    def piece(G, t):
        w = jnp.concatenate([weight(WO0, 2 * G + r) for r in range(2)], axis=1)
        acc[t, _ds(G >> 3, D, 64), :] += _dot_nt(w, o_vm[t * 128:(t + 1) * 128, :])

    def pairs(G0, count, step, first, cells):
        for u in range(count):
            slots = slots_of(G0 + u)
            pl.when(G0 + u >= NG)(lambda: wait_slot(slots[1]))
            wait_slot(slots[0])
        if count == 2:
            wait_w(WO0, 2 * G0, 4, s_wo.at[G0 >> 1])
        else:
            pl.when((G0 & 1) == 0)(lambda: wait_w(WO0, 2 * G0, 4, s_wo.at[G0 >> 1]))

        def qk(n):
            u, j = divmod(n, 2 * NB)
            b, r = divmod(j, 2)
            return _dot_nt(q_vm[2 * (G0 + u) + r, b * SQ:(b + 1) * SQ], buf[_ring(slots_of(G0 + u)[r], 0, b)])

        tick = _spreader(count * 4 * NB, lambda part, k: start_nth(part, first[_queue(part)], k),
                         [2 * c for c in cells])
        for j in range(NF):
            q_fin[j, _ds(step, SQ, 16)] = qproj(2 * NMAIN + j, _ds(step, SQ, 16))
        s_next = qk(0)
        for n in range(count * 2 * NB):
            u, j = divmod(n, 2 * NB)
            b, r = divmod(j, 2)
            s = s_next
            if n + 1 < count * 2 * NB:
                s_next = qk(n + 1)
            tick()
            p, inv = _softmax_parts(s)
            if r == 1 and b >= 3:
                piece(G0 + u, b - 3)
            if r == 1 and b < 2 and u > 0:
                piece(G0 + u - 1, NPIECE - 2 + b)
            o = _dot(p, buf[_ring(slots_of(G0 + u)[r], 1, b)]) * inv
            o_vm[b * SQ:(b + 1) * SQ, r * DH:(r + 1) * DH] = o.astype(BF16)
            tick()
        piece(G0 + count - 1, NPIECE - 2)
        piece(G0 + count - 1, NPIECE - 1)

    nsingle = NMAIN - 2 * NDOUBLE
    m0 = [NQ * c for c in QC]
    m1 = [m + NDOUBLE * c for m, c in zip(m0, C2)]
    m2 = [m + nsingle * c - NKV * NB for m, c in zip(m1, C1)]
    assert NDOUBLE + nsingle == NB and all(m % NF == 0 for m in m2)
    for q in range(2):
        assert all(m0[q] + i * C2[q] >= NB * max(2 * i + 2, 4 * i + 4 - NG) for i in range(NDOUBLE))
        assert all(m1[q] + i * C1[q] >= NB * (4 * NDOUBLE - NG + 2 * i + 2) for i in range(nsingle))
        assert all(m0[q] + (i + 1) * C2[q] <= NB * (NS + min(max(2 * i, 4 * i - NG), NKV - NS)) for i in range(NDOUBLE - 1))
        assert 4 * (NDOUBLE - 1) - NG >= NS
    pl.loop(0, NDOUBLE)(lambda i: pairs(2 * i, 2, i, [m + i * c for m, c in zip(m0, C2)], C2))
    pl.loop(0, nsingle)(
        lambda i: pairs(2 * NDOUBLE + i, 1, NDOUBLE + i, [m + i * c for m, c in zip(m1, C1)], C1))

    def qk_fin(b, j):
        return _dot_nt(q_fin[j, b * SQ:(b + 1) * SQ], buf[_fin(b, 0, j)])

    def pv_fin(b, j, p, inv):
        fin_vm[b * SQ:(b + 1) * SQ, j * DH:(j + 1) * DH] = (_dot(p, buf[_fin(b, 1, j)]) * inv).astype(BF16)

    def oproj_fin(t, c0=D, c1=2 * D):
        w = jnp.concatenate([buf[WO0 + 2 * NMAIN + j, c0 - D:c1 - D] for j in range(NF)], axis=1)
        return acc[t, c0:c1, :] + _dot_nt(w, fin_vm[t * 128:(t + 1) * 128, :OUT0])

    def emit(t, n=2 * D):
        fin_vm[t * 128:(t + 1) * 128, OUT0:OUT0 + n] = acc[t, :n, :].T.astype(BF16)

    issued = [2 * m2[_queue(part)] for part in range(NH + 1)]

    def start_late(part, _):
        b, isv, j = issued[part] // (2 * NF), issued[part] // NF % 2, issued[part] % NF
        if part < NH or j == 0:
            start_fin(part, b, isv, j)
        issued[part] += 1

    wait_w(WO0, 2 * NMAIN, NF, s_wo.at[NMAIN // 2])
    done = emitted = sent = 0
    for lo, hi, send, nxt, ticks in STAGES:
        assert min(issued) >= hi * NF
        for n in range(lo, hi):
            _wait_all(buf.at[pl.ds(_fin(n // 2, n % 2, 0), NF)], s_kv.at[NS + n])
        if hi == 2 * NB:
            cp_last(0).start()

        def flush():
            nonlocal sent
            while sent < min(send, emitted):
                cp_out(sent).start(priority=sent % 2)
                sent += 1

        def finish():
            nonlocal emitted
            while emitted < done:
                emit(emitted)
                emitted += 1
            flush()
            if lo == 0:
                emit(NPIECE - 1, 384)

        flush()
        tick = _spreader(ticks, start_late,
                         [nxt * NF - issued[0], min(nxt + LEAD, 2 * NB) * NF - issued[NH]])
        if lo % 2:
            for j in range(NF):
                tick()
                pv_fin(lo // 2, j, p_vm[j], jnp.concatenate([inv_vm[j]] * (DH // 128), axis=1))
                if j == 1:
                    finish()
        units = [(n // 2, j) for n in range(lo, hi) if n % 2 == 0 for j in range(NF)]
        have = (lo + 1) // 2
        limit = (hi - 1) // 2 - 1
        if units:
            s_next = qk_fin(*units[0])
        for i, (b, j) in enumerate(units):
            s = s_next
            if i + 1 < len(units):
                s_next = qk_fin(*units[i + 1])
            tick()
            p, inv = _softmax_parts(s)
            keep = 2 * b + 1 == hi
            if keep:
                p_vm[j] = p
                inv_vm[j] = jnp.broadcast_to(inv, (SQ, 128))
            if j == NF - 1 and done < min(have - 1, limit):
                acc[done, D:, :] = oproj_fin(done)
                done += 1
            if not keep:
                pv_fin(b, j, p, inv)
                have += j == NF - 1
            if i == 1 and lo % 2 == 0:
                finish()
            tick()
        while done < limit:
            acc[done, D:, :] = oproj_fin(done)
            done += 1
    assert done == emitted == sent == NPIECE - 1
    for i, (c0, c1) in enumerate(((D, 640), (640, 2 * D))):
        r = oproj_fin(NPIECE - 1, c0, c1)
        if i == 0:
            r = jnp.concatenate([acc[NPIECE - 1, 384:D, :], r], axis=0)
        fin_vm[M - 128:, OUT0 + c1 - 256:OUT0 + c1] = r.T.astype(BF16)
        cp_last(1 + i).start(priority=1 - i)

    for t in range(NPIECE - 1):
        cp_out(t).wait()
    for i in range(3):
        cp_last(i).wait()


@jax.jit
def pallas_concat_heads__gqa_block_cached__mha_block_cached__near_ridge_kernel(
    A_x: jax.Array,
    A_k_cache: jax.Array,
    A_v_cache: jax.Array,
    A_wq: jax.Array,
    A_wo: jax.Array,
    B_x: jax.Array,
    B_k_cache: jax.Array,
    B_v_cache: jax.Array,
    B_wq: jax.Array,
    B_wo: jax.Array,
):
    out = pl.pallas_call(
        _kernel,
        out_shape=jax.ShapeDtypeStruct((M, 2 * D), BF16),
        in_specs=[pl.BlockSpec(memory_space=pl.ANY)] * 10,
        out_specs=pl.BlockSpec(memory_space=pl.ANY),
        scratch_shapes=[
            pltpu.VMEM((2, M, D), BF16),
            pltpu.VMEM((WO0 + 2 * HQ, SK, DH), BF16),
            pltpu.VMEM((2 * NMAIN, M, DH), BF16),
            pltpu.VMEM((NF, M, DH), BF16),
            pltpu.VMEM((M, 2 * DH), BF16),
            pltpu.VMEM((M, OUT0 + 2 * D), BF16),
            pltpu.VMEM((NF, SQ, SK), BF16),
            pltpu.VMEM((NF, SQ, 128), F32),
            pltpu.VMEM((NPIECE, 2 * D, 128), F32),
            pltpu.SemaphoreType.DMA((len(XCUT),)),
            pltpu.SemaphoreType.DMA((3 + NQ,)),
            pltpu.SemaphoreType.DMA((NG,)),
            pltpu.SemaphoreType.DMA((NS + 2 * NB,)),
            pltpu.SemaphoreType.DMA((NPIECE + 2,)),
        ],
        compiler_params=pltpu.CompilerParams(
            vmem_limit_bytes=120 * 2**20, disable_bounds_checks=True, disable_semaphore_checks=True),
    )(A_x.reshape(M, D), A_k_cache, A_v_cache, A_wq, A_wo.T,
      B_x.reshape(M, D), B_k_cache, B_v_cache, B_wq, B_wo.T)
    return out.reshape(NB, SQ, 2 * D)
```
